```python
import os as _os
_os.environ.setdefault("JAX_PLATFORMS", "cpu")
import jax
import jax.numpy as jnp

def _softmax(x, axis=-1):
    return jax.nn.softmax(x, axis=axis)
def _gelu(x):
    return jax.nn.gelu(x, approximate=True)
def _silu(x):
    return jax.nn.silu(x)
def _sigmoid(x):
    return jax.nn.sigmoid(x)
def _layernorm(x, axis=-1, eps=1e-5):
    m = jnp.mean(x, axis=axis, keepdims=True)
    v = jnp.var(x, axis=axis, keepdims=True)
    return (x - m) / jnp.sqrt(v + eps)
def _scatter_add(tgt, idx, src, axis=0):
    return tgt.at[idx].add(src)
def _segment_sum(src, seg, n):
    return jax.ops.segment_sum(src, seg, n)
class _Rng:
    def __init__(self, key):
        self._k = key
    def _next(self):
        self._k, sub = jax.random.split(self._k)
        return sub
    def normal(self, shape):
        return jax.random.normal(self._next(), shape, dtype=jnp.bfloat16)
    def randint(self, lo, hi, shape):
        return jax.random.randint(self._next(), shape, lo, hi, dtype=jnp.int32)
    def uniform(self, shape, lo=0.0, hi=1.0):
        return jax.random.uniform(self._next(), shape, jnp.bfloat16, lo, hi)
    def permutation(self, n):
        return jax.random.permutation(self._next(), n)


kernel_name = 'gated_mix__grouped_kv_mqa__ssm_conv_s5__prompt'

def setup_inputs():
    _rng = _Rng(jax.random.key(int.from_bytes(__import__("os").urandom(4), "little")))
    _w = (lambda a: (lambda t: t.astype(jnp.bfloat16) if jnp.issubdtype(t.dtype, jnp.floating) else t)(jnp.asarray(a)))
    def _A_setup():
        B, S, D, H = 1, 2048, 512, 32
        Dh = D // H
        return {
            "x": _w((lambda *s: _rng.normal(s) * 0.05)(B, S, D)),
            "wq": _w((lambda *s: _rng.normal(s) * 1.6)(D, H * Dh)),
            "wk": _w((lambda *s: _rng.normal(s) * 1.6)(D, Dh)),
            "wv": _w((lambda *s: _rng.normal(s) * 0.05)(D, Dh)),
            "wo": _w((lambda *s: _rng.normal(s) * 0.05)(H * Dh, D)),
        }
    _A_in = _A_setup()

    def _B_setup():
        B, S, D = 1, 2048, 512
        P = D
        Lambda_re = -0.5 * jnp.exp((lambda *s: _rng.normal(s) * 0.4)(P))
        Lambda_im = (lambda *s: _rng.normal(s) * 0.4)(P) * 1.0
        B_re = (lambda *s: _rng.normal(s) * 0.4)(P, D) * (D ** -0.5)
        B_im = (lambda *s: _rng.normal(s) * 0.4)(P, D) * (D ** -0.5)
        C_re = (lambda *s: _rng.normal(s) * 0.4)(D, P) * (P ** -0.5)
        C_im = (lambda *s: _rng.normal(s) * 0.4)(D, P) * (P ** -0.5)
        log_dt = (lambda *s: _rng.normal(s) * 0.4)(P) * 0.3 - 2.0
        Dskip = (lambda *s: _rng.normal(s) * 0.4)(D)
        return {
            "x": _w((lambda *s: _rng.normal(s) * 0.05)(B, S, D)),
            "Lambda_re": _w(Lambda_re),
            "Lambda_im": _w(Lambda_im),
            "B_re": _w(B_re),
            "B_im": _w(B_im),
            "C_re": _w(C_re),
            "C_im": _w(C_im),
            "log_dt": _w(log_dt),
            "Dskip": _w(Dskip),
        }
    _B_in = _B_setup()

    return {
        "A_x": _A_in["x"],
        "A_wq": _A_in["wq"],
        "A_wk": _A_in["wk"],
        "A_wv": _A_in["wv"],
        "A_wo": _A_in["wo"],
        "B_x": _B_in["x"],
        "B_Lambda_re": _B_in["Lambda_re"],
        "B_Lambda_im": _B_in["Lambda_im"],
        "B_B_re": _B_in["B_re"],
        "B_B_im": _B_in["B_im"],
        "B_C_re": _B_in["C_re"],
        "B_C_im": _B_in["C_im"],
        "B_log_dt": _B_in["log_dt"],
        "B_Dskip": _B_in["Dskip"],
        "gate_w": _w((lambda *s: _rng.normal(s) * 0.05)(512) * 16.0),
    }

def reference(A_x, A_wq, A_wk, A_wv, A_wo, B_x, B_Lambda_re, B_Lambda_im, B_B_re, B_B_im, B_C_re, B_C_im, B_log_dt, B_Dskip, gate_w):
    def _A_ref(x, wq, wk, wv, wo):
        B, S, D = x.shape
        H = 32
        Dh = D // H
        q = (lambda x, *d: x.transpose(*d))((x @ wq).reshape(B, S, H, Dh), 0, 2, 1, 3)
        k = x @ wk
        v = x @ wv
        scores = jnp.einsum("bhqd,bkd->bhqk", q, k) * (Dh ** -0.5)
        p = _softmax(scores, axis=-1)
        o = jnp.einsum("bhqk,bkd->bhqd", p, v)
        return (lambda x, *d: x.transpose(*d))(o, 0, 2, 1, 3).reshape(B, S, H * Dh) @ wo

    def _B_ref(x, Lambda_re, Lambda_im, B_re, B_im, C_re, C_im, log_dt, Dskip):
        Bsz, L, H = x.shape
        Lam = Lambda_re + 1j * Lambda_im
        Bmat = B_re + 1j * B_im
        Cmat = C_re + 1j * C_im
        dt = jnp.exp(log_dt)
        Lam_bar = jnp.exp(dt * Lam)
        B_bar = ((Lam_bar - 1.0) / Lam)[:, None] * Bmat
        Bu = jnp.einsum("bld,pd->blp", x + 0j, B_bar)
        h = jnp.zeros_like(Bu[:, 0, :])
        hs = []
        for t in range(L):
            h = Lam_bar[None, :] * h + Bu[:, t, :]
            hs.append(h)
        hseq = jnp.stack(hs, 1)
        y = 2.0 * jnp.einsum("blp,dp->bld", hseq, Cmat).real + x * Dskip[None, None, :]
        return y

    x = A_x
    g = _sigmoid((x * gate_w).sum(-1, keepdims=True))
    a = _A_ref(x, A_wq, A_wk, A_wv, A_wo)
    b = _B_ref(x, B_Lambda_re, B_Lambda_im, B_B_re, B_B_im, B_C_re, B_C_im, B_log_dt, B_Dskip)
    return g * a + (1 - g) * b
```

```python
import numpy as np
import jax
import jax.numpy as jnp
from jax import lax
import jax.experimental.pallas as pl
import jax.experimental.pallas.tpu as pltpu

S, D, H, DH, P = 2048, 512, 32, 16, 512
BQ = 512
NB = S // BQ
BK = 128
NKB = S // BK
LA = 2
U = 8
NCH = 8
TCH = BQ // NCH
PITCH = TCH + 8
NP = P // 128
RC = 128
EMBED = 1
STAGGER = 0
QSCALE = float(np.log2(np.e) * DH ** -0.5)
UP = 1.0 + 2.0 ** -7
L_MIN = 2.0 ** -64
F32, BF16 = jnp.float32, jnp.bfloat16
NT = (((1,), (1,)), ((), ()))


def _dot(a, b):
    return jnp.dot(a, b, preferred_element_type=F32)


def _dot_nt(a, b):
    return lax.dot_general(a, b, NT, preferred_element_type=F32)


def _cmul(ar, ai, br, bi):
    return ar * br - ai * bi, ar * bi + ai * br


def _kernel(x_hbm, wq_hbm, wk_hbm, wv_hbm, wo_hbm, lre_hbm, lim_hbm, bre_hbm, bim_hbm,
            cre_hbm, cim_hbm, ldt_hbm, dsk_hbm, gw_hbm, o_hbm,
            x_s, wq_s, wk_s, wv_s, wo_s, lre_s, lim_s, bre_s, bim_s, cre_s, cim_s, ldt_s, dsk_s, gw_s,
            qa_s, ka_s, vt_s, kt_s, ot_s, u_s, st_s, coef_s, pw_s, carry_s, ob_s, isem, osem):
    cp = lambda src, dst, n: pltpu.make_async_copy(src, dst, isem.at[n])
    c_wq = cp(wq_hbm, wq_s, 0)
    c_wk = cp(wk_hbm, wk_s, 1)
    c_wv = cp(wv_hbm, wv_s, 2)
    c_x = [cp(x_hbm.at[pl.ds(t * BQ, BQ)], x_s.at[pl.ds(t * BQ, BQ)], 3 + t) for t in range(NB)]
    c_vec = [cp(a, b, 7 + n) for n, (a, b) in enumerate(
        ((lre_hbm, lre_s), (lim_hbm, lim_s), (ldt_hbm, ldt_s), (dsk_hbm, dsk_s), (gw_hbm, gw_s)))]
    c_big = [cp(a, b, 12 + n) for n, (a, b) in enumerate(
        ((bre_hbm, bre_s), (bim_hbm, bim_s), (cre_hbm, cre_s), (cim_hbm, cim_s), (wo_hbm, wo_s)))]
    for c in [c_wq, c_wk, c_wv] + c_x + c_vec:
        c.start()
    if not STAGGER:
        for c in c_big:
            c.start()

    c_wq.wait()
    wqT = wq_s[...].astype(F32).T.astype(BF16)
    c_wk.wait()
    c_wv.wait()
    lhs = jnp.concatenate([wqT, wk_s[...], wv_s[...]], axis=0)
    for tb in range(NB):
        c_x[tb].wait()
        if STAGGER and tb == NB - 1:
            for c in c_big:
                c.start()
        r = _dot_nt(lhs, x_s[tb * BQ:(tb + 1) * BQ, :])
        q = (r[:D] * QSCALE).astype(BF16)
        qf = q.astype(F32)
        for h in range(H):
            a = qf[h * DH:h * DH + 8]
            b = qf[h * DH + 8:(h + 1) * DH]
            n = a * a + b * b
            n = n + pltpu.roll(n, 4, 0)
            n = n + pltpu.roll(n, 2, 0)
            n = n + pltpu.roll(n, 1, 0)
            nrm = -(jnp.sqrt(n) * UP)
            qa_s[tb, h, 0:DH, :] = q[h * DH:(h + 1) * DH]
            qa_s[tb, h, DH:2 * DH, :] = jnp.concatenate([nrm, nrm], axis=0).astype(BF16)
        kt_s[:, tb * BQ:(tb + 1) * BQ] = r[D:D + DH].astype(BF16).astype(F32)
        vt_s[:, tb * BQ:(tb + 1) * BQ] = r[D + DH:D + 2 * DH].astype(BF16)
    kt = kt_s[...]
    k2 = jnp.sum(kt * kt, axis=0, keepdims=True)
    kmax = jnp.sqrt(jnp.max(k2, axis=1, keepdims=True)) * UP
    kcol = (kmax.astype(BF16).astype(F32) * (1.0 / DH))
    for kb in range(NKB):
        kta = jnp.concatenate([kt[:, kb * BK:(kb + 1) * BK],
                               jnp.broadcast_to(kcol, (DH, BK)),
                               jnp.zeros((128 - 2 * DH, BK), F32)], axis=0)
        ka_s[kb] = kta.T.astype(BF16)

    for c in c_vec:
        c.wait()
    vec8 = lambda ref: jnp.broadcast_to(ref[...].astype(F32).reshape(1, P), (8, P))
    lre, lim = vec8(lre_s), vec8(lim_s)
    dt = jnp.exp(vec8(ldt_s)).astype(BF16).astype(F32)
    er = jnp.exp(dt * lre)
    lr = er * jnp.cos(dt * lim)
    li = er * jnp.sin(dt * lim)
    den = lre * lre + lim * lim
    nr = lr - 1.0
    coef_s[0] = lr
    coef_s[1] = li
    coef_s[2] = 2.0 * (nr * lre + li * lim) / den
    coef_s[3] = 2.0 * (li * lre - nr * lim) / den
    row = lax.broadcasted_iota(jnp.int32, (NCH, P), 0)
    pr, pi = lr, li
    ar, ai = lr, li
    for k in range(3):
        tr, ti = _cmul(pr, pi, ar, ai)
        sel = (row & (1 << k)) != 0
        pr, pi = jnp.where(sel, tr, pr), jnp.where(sel, ti, pi)
        ar, ai = _cmul(ar, ai, ar, ai)
    for g in range(TCH // 8):
        pw_s[0, g * 8:(g + 1) * 8, :] = pr
        pw_s[1, g * 8:(g + 1) * 8, :] = pi
        pr, pi = _cmul(pr, pi, ar, ai)
    for _ in range(3):
        ar, ai = _cmul(ar, ai, ar, ai)
    for j in range(3):
        coef_s[4 + 2 * j] = ar
        coef_s[5 + 2 * j] = ai
        ar, ai = _cmul(ar, ai, ar, ai)
    coef_s[10] = vec8(dsk_s)
    coef_s[11] = vec8(gw_s)
    carry_s[...] = jnp.zeros_like(carry_s)
    for c in c_big:
        c.wait()

    zpad = jnp.zeros((128 - 2 * DH, BQ), BF16)

    def out_copy(i, r):
        return pltpu.make_async_copy(
            ob_s.at[pl.ds(r * RC, RC)],
            o_hbm.at[pl.ds(pl.multiple_of(i * BQ, BQ) + r * RC, RC)], osem.at[r])

    def scan_steps(t0, n):
        hr = [st_s[0, j] for j in range(NP)]
        hi = [st_s[1, j] for j in range(NP)]
        for dt_ in range(n):
            t = t0 + dt_
            for j in range(NP):
                lr_, li_ = coef_s[0, :, j * 128:(j + 1) * 128], coef_s[1, :, j * 128:(j + 1) * 128]
                a = u_s[0, j, pl.ds(t, NCH, stride=PITCH), :]
                b = u_s[1, j, pl.ds(t, NCH, stride=PITCH), :]
                nr_ = lr_ * hr[j] - li_ * hi[j] + a
                ni_ = lr_ * hi[j] + li_ * hr[j] + b
                hr[j], hi[j] = nr_, ni_
                u_s[0, j, pl.ds(t, NCH, stride=PITCH), :] = nr_
                u_s[1, j, pl.ds(t, NCH, stride=PITCH), :] = ni_
        for j in range(NP):
            st_s[0, j] = hr[j]
            st_s[1, j] = hi[j]

    def qblock(i, _):
        xb = x_s[pl.ds(pl.multiple_of(i * BQ, BQ), BQ), :]
        ur = _dot_nt(xb, bre_s[...])
        ui = _dot_nt(xb, bim_s[...])
        cr = jnp.broadcast_to(coef_s[2, 0:1, :], (BQ, P))
        ci = jnp.broadcast_to(coef_s[3, 0:1, :], (BQ, P))
        bur = cr * ur - ci * ui
        bui = cr * ui + ci * ur
        for j in range(NP):
            for c in range(NCH):
                u_s[0, j, c * PITCH:c * PITCH + TCH, :] = bur[c * TCH:(c + 1) * TCH, j * 128:(j + 1) * 128]
                u_s[1, j, c * PITCH:c * PITCH + TCH, :] = bui[c * TCH:(c + 1) * TCH, j * 128:(j + 1) * 128]
        st_s[...] = jnp.zeros_like(st_s)
        if not EMBED:
            def sb(t, _):
                scan_steps(t * 8, 8)
                return 0
            lax.fori_loop(0, TCH // 8, sb, 0)

        def finish(h, acc, l8, bad):
            l = jnp.sum(l8, axis=0, keepdims=True)
            ot_s[h] = acc * (1.0 / l)
            return jnp.maximum(bad, jnp.where(l >= L_MIN, 0.0, 1.0))

        def heads_body(hg, bad):
            nst = U * NKB
            spi = TCH // (H // U)
            qw = {}

            def qk(t):
                u, kb = divmod(t, NKB)
                if u not in qw:
                    qw[u] = jnp.concatenate([qa_s[i, hg * U + u], zpad], axis=0)
                return _dot(ka_s[kb], qw[u])

            ss = {t: qk(t) for t in range(LA)}
            acc = l8 = None
            for t in range(nst):
                u, kb = divmod(t, NKB)
                if t + LA < nst:
                    ss[t + LA] = qk(t + LA)
                p = jnp.exp2(ss.pop(t))
                ps = p.reshape(BK // 8, 8, BQ).sum(axis=0)
                pv = _dot(vt_s[:, kb * BK:(kb + 1) * BK], p.astype(BF16))
                if kb == 0:
                    acc, l8 = pv, ps
                else:
                    acc, l8 = acc + pv, l8 + ps
                if kb == NKB - 1:
                    bad = finish(hg * U + u, acc, l8, bad)
                if EMBED and kb == NKB // 2:
                    n = spi // U
                    scan_steps(hg * spi + u * n, n)
            return bad

        bad = lax.fori_loop(0, H // U, heads_body, jnp.zeros((1, BQ), F32))

        @pl.when(jnp.max(bad) > 0.0)
        def _exact_softmax():
            lane = lax.broadcasted_iota(jnp.int32, (BK, 128), 1)

            def head(h, _):
                qw = jnp.concatenate([qa_s[i, h, 0:DH, :], jnp.zeros((128 - DH, BQ), BF16)], axis=0)

                def kb_body(kb, c):
                    m, l, acc = c
                    ka = jnp.where(lane < DH, ka_s[kb], jnp.zeros((BK, 128), BF16))
                    s = _dot(ka, qw)
                    m_new = jnp.maximum(m, jnp.max(s, axis=0, keepdims=True))
                    alpha = jnp.exp2(m - m_new)
                    p = jnp.exp2(s - m_new)
                    l = alpha * l + jnp.sum(p, axis=0, keepdims=True)
                    vt = vt_s[:, pl.ds(pl.multiple_of(kb * BK, BK), BK)]
                    acc = alpha * acc + _dot(vt, p.astype(BF16))
                    return m_new, l, acc

                m, l, acc = lax.fori_loop(
                    0, NKB, kb_body,
                    (jnp.full((1, BQ), -jnp.inf, F32), jnp.zeros((1, BQ), F32), jnp.zeros((DH, BQ), F32)))
                ot_s[h] = acc * (1.0 / l)
                return 0

            lax.fori_loop(0, H, head, 0)

        er = jnp.concatenate([st_s[0, j] for j in range(NP)], axis=1)
        ei = jnp.concatenate([st_s[1, j] for j in range(NP)], axis=1)
        c_r, c_i = carry_s[0], carry_s[1]
        tr, ti = _cmul(coef_s[4], coef_s[5], c_r, c_i)
        er = er + jnp.where(row == 0, tr, 0.0)
        ei = ei + jnp.where(row == 0, ti, 0.0)
        for j, d in enumerate((1, 2, 4)):
            sr = jnp.where(row >= d, pltpu.roll(er, d, 0), 0.0)
            si = jnp.where(row >= d, pltpu.roll(ei, d, 0), 0.0)
            tr, ti = _cmul(coef_s[4 + 2 * j], coef_s[5 + 2 * j], sr, si)
            er, ei = er + tr, ei + ti
        carry_s[0] = jnp.broadcast_to(er[NCH - 1:NCH], (NCH, P))
        carry_s[1] = jnp.broadcast_to(ei[NCH - 1:NCH], (NCH, P))
        e0r = jnp.where(row == 0, c_r, pltpu.roll(er, 1, 0))
        e0i = jnp.where(row == 0, c_i, pltpu.roll(ei, 1, 0))

        pwr, pwi = pw_s[0], pw_s[1]
        dsk = coef_s[10, 0:1, :]
        gw = coef_s[11, 0:1, :]
        for r in range(BQ // RC):
            hrs, his = [], []
            for c in range(r * RC // TCH, (r + 1) * RC // TCH):
                gr = jnp.concatenate([u_s[0, j, c * PITCH:c * PITCH + TCH, :] for j in range(NP)], axis=1)
                gi = jnp.concatenate([u_s[1, j, c * PITCH:c * PITCH + TCH, :] for j in range(NP)], axis=1)
                br = jnp.broadcast_to(e0r[c:c + 1], (TCH, P))
                bi = jnp.broadcast_to(e0i[c:c + 1], (TCH, P))
                tr, ti = _cmul(pwr, pwi, br, bi)
                hrs.append((gr + tr).astype(BF16))
                his.append((gi + ti).astype(BF16))
            hr = jnp.concatenate(hrs, axis=0)
            hi = jnp.concatenate(his, axis=0)
            y = _dot_nt(hr, cre_s[...]) - _dot_nt(hi, cim_s[...])
            xf = x_s[pl.ds(pl.multiple_of(i * BQ, BQ) + r * RC, RC), :].astype(F32)
            bb = y + xf * dsk
            g = jax.nn.sigmoid(jnp.sum(xf * gw, axis=1, keepdims=True))
            o = ot_s[:, :, r * RC:(r + 1) * RC].reshape(H * DH, RC).T.astype(BF16)
            a = _dot(o, wo_s[...])

            @pl.when(i > 0)
            def _():
                out_copy(i - 1, r).wait()

            ob_s[r * RC:(r + 1) * RC, :] = g * a + (1.0 - g) * bb
            out_copy(i, r).start()
        return 0

    lax.fori_loop(0, NB, qblock, 0)
    for r in range(BQ // RC):
        out_copy(NB - 1, r).wait()


@jax.jit
def pallas_gated_mix__grouped_kv_mqa__ssm_conv_s5__prompt_kernel(
    A_x, A_wq, A_wk, A_wv, A_wo, B_x, B_Lambda_re, B_Lambda_im, B_B_re, B_B_im,
    B_C_re, B_C_im, B_log_dt, B_Dskip, gate_w,
):
    x = A_x.reshape(S, D)
    args = (x, A_wq, A_wk.T, A_wv.T, A_wo, B_Lambda_re, B_Lambda_im, B_B_re, B_B_im,
            B_C_re, B_C_im, B_log_dt, B_Dskip, gate_w)
    out = pl.pallas_call(
        _kernel,
        in_specs=[pl.BlockSpec(memory_space=pl.ANY)] * len(args),
        out_specs=pl.BlockSpec(memory_space=pl.ANY),
        out_shape=jax.ShapeDtypeStruct((S, D), F32),
        scratch_shapes=[pltpu.VMEM(a.shape, a.dtype) for a in args] + [
            pltpu.VMEM((NB, H, 2 * DH, BQ), BF16),
            pltpu.VMEM((NKB, BK, 128), BF16),
            pltpu.VMEM((DH, S), BF16),
            pltpu.VMEM((DH, S), F32),
            pltpu.VMEM((H, DH, BQ), F32),
            pltpu.VMEM((2, NP, NCH * PITCH, 128), F32),
            pltpu.VMEM((2, NP, NCH, 128), F32),
            pltpu.VMEM((12, 8, P), F32),
            pltpu.VMEM((2, TCH, P), F32),
            pltpu.VMEM((2, 8, P), F32),
            pltpu.VMEM((BQ, D), F32),
            pltpu.SemaphoreType.DMA((17,)),
            pltpu.SemaphoreType.DMA((BQ // RC,)),
        ],
        compiler_params=pltpu.CompilerParams(vmem_limit_bytes=100 * 1024 * 1024),
        name="gmix",
    )(*args)
    return out.reshape(1, S, D)
```

```python
import numpy as np
import jax
import jax.numpy as jnp
from jax import lax
import jax.experimental.pallas as pl
import jax.experimental.pallas.tpu as pltpu

S, D, H, DH, P = 2048, 512, 32, 16, 512
BQ = 512
NB = S // BQ
BK = 128
NKB = S // BK
LA = 2
U = 16
NIT = H // U
NCH = 8
TCH = BQ // NCH
SPI = TCH // NIT
SUB = 16
PITCH = TCH + 8
UPITCH = SUB + 8
NP = P // 128
RC = 128
T_SSM = 2
T_SCAN = NKB // 2
QSCALE = float(np.log2(np.e) * DH ** -0.5)
UP = 1.0 + 2.0 ** -7
L_MIN = 2.0 ** -64
F32, BF16 = jnp.float32, jnp.bfloat16
NT = (((1,), (1,)), ((), ()))


def _dot(a, b):
    return jnp.dot(a, b, preferred_element_type=F32)


def _dot_nt(a, b):
    return lax.dot_general(a, b, NT, preferred_element_type=F32)


def _cmul(ar, ai, br, bi):
    return ar * br - ai * bi, ar * bi + ai * br


def _kernel(x_hbm, wq_hbm, wk_hbm, wv_hbm, wo_hbm, lre_hbm, lim_hbm, bre_hbm, bim_hbm,
            cre_hbm, cim_hbm, ldt_hbm, dsk_hbm, gw_hbm, o_hbm,
            x_s, wq_s, wk_s, wv_s, wo_s, lre_s, lim_s, bre_s, bim_s, cre_s, cim_s, ldt_s, dsk_s, gw_s,
            qa_s, ka_s, vt_s, km_s, ot_s, u_s, g_s, st_s, coef_s, pw_s, carry_s, ob_s, p_s, l_s,
            isem, osem):
    def cp(src, dst, n):
        return pltpu.make_async_copy(src, dst, isem.at[n])

    c_wq, c_wk, c_wv = cp(wq_hbm, wq_s, 0), cp(wk_hbm, wk_s, 1), cp(wv_hbm, wv_s, 2)
    c_x = [cp(x_hbm.at[pl.ds(t * BQ, BQ)], x_s.at[pl.ds(t * BQ, BQ)], 3 + t) for t in range(NB)]
    c_vec = [cp(a, b, 3 + NB + n) for n, (a, b) in enumerate(
        ((lre_hbm, lre_s), (lim_hbm, lim_s), (ldt_hbm, ldt_s), (dsk_hbm, dsk_s), (gw_hbm, gw_s)))]
    c_big = [cp(a, b, 8 + NB + n) for n, (a, b) in enumerate(
        ((bre_hbm, bre_s), (bim_hbm, bim_s), (cre_hbm, cre_s), (cim_hbm, cim_s), (wo_hbm, wo_s)))]
    for c in c_vec + [c_wq, c_wk, c_wv] + c_x + c_big:
        c.start()

    for c in c_vec:
        c.wait()

    def vec8(ref):
        return jnp.broadcast_to(ref[...].astype(F32).reshape(1, P), (8, P))

    lre, lim = vec8(lre_s), vec8(lim_s)
    dt = jnp.exp(vec8(ldt_s)).astype(BF16).astype(F32)
    er = jnp.exp(dt * lre)
    lr = er * jnp.cos(dt * lim)
    li = er * jnp.sin(dt * lim)
    den = lre * lre + lim * lim
    nr = lr - 1.0
    coef_s[0] = lr
    coef_s[1] = li
    coef_s[2] = 2.0 * (nr * lre + li * lim) / den
    coef_s[3] = 2.0 * (li * lre - nr * lim) / den
    row = lax.broadcasted_iota(jnp.int32, (NCH, P), 0)
    pr, pi = lr, li
    ar, ai = lr, li
    for k in range(3):
        tr, ti = _cmul(pr, pi, ar, ai)
        sel = (row & (1 << k)) != 0
        pr, pi = jnp.where(sel, tr, pr), jnp.where(sel, ti, pi)
        ar, ai = _cmul(ar, ai, ar, ai)
    for g in range(TCH // 8):
        pw_s[0, g * 8:(g + 1) * 8, :] = pr
        pw_s[1, g * 8:(g + 1) * 8, :] = pi
        pr, pi = _cmul(pr, pi, ar, ai)
    for _ in range(3):
        ar, ai = _cmul(ar, ai, ar, ai)
    for j in range(3):
        coef_s[4 + 2 * j] = ar
        coef_s[5 + 2 * j] = ai
        ar, ai = _cmul(ar, ai, ar, ai)
    coef_s[10] = vec8(dsk_s)
    coef_s[11] = vec8(gw_s)
    carry_s[...] = jnp.zeros_like(carry_s)

    c_wq.wait()
    c_wk.wait()
    c_wv.wait()
    c_x[0].wait()
    wqT = wq_s[...].astype(F32).T.astype(BF16)
    lhs = jnp.concatenate([wk_s[...], wv_s[...], wqT], axis=0)
    k2max = None
    for tb in range(NB):
        if tb == 1:
            for c in c_x[1:]:
                c.wait()
        r = _dot_nt(lhs, x_s[tb * BQ:(tb + 1) * BQ, :])
        q = (r[2 * DH:] * QSCALE).astype(BF16)
        qf = q.astype(F32)
        for h in range(H):
            a = qf[h * DH:h * DH + 8]
            b = qf[h * DH + 8:(h + 1) * DH]
            n = a * a + b * b
            n = n + pltpu.roll(n, 4, 0)
            n = n + pltpu.roll(n, 2, 0)
            n = n + pltpu.roll(n, 1, 0)
            nrm = -(jnp.sqrt(n) * UP)
            qa_s[tb * H + h, 0:DH, :] = q[h * DH:(h + 1) * DH]
            qa_s[tb * H + h, DH:2 * DH, :] = jnp.concatenate([nrm, nrm], axis=0).astype(BF16)
        kt = r[0:DH].astype(BF16).astype(F32)
        vt_s[:, tb * BQ:(tb + 1) * BQ] = r[DH:2 * DH].astype(BF16)
        k2 = jnp.sum(kt * kt, axis=0, keepdims=True)
        k2max = k2 if k2max is None else jnp.maximum(k2max, k2)
        for kb in range(BQ // BK):
            kta = jnp.concatenate([kt[:, kb * BK:(kb + 1) * BK],
                                   jnp.full((DH, BK), 1.0 / DH, F32),
                                   jnp.zeros((128 - 2 * DH, BK), F32)], axis=0)
            ka_s[tb * (BQ // BK) + kb] = kta.T.astype(BF16)
    kmax = jnp.sqrt(jnp.max(k2max, axis=1, keepdims=True)) * UP
    km_s[...] = jnp.broadcast_to(kmax, (8, 128))

    zpad = jnp.zeros((128 - 2 * DH, BQ), BF16)

    def q_weights(fh):
        km = jnp.concatenate([km_s[...]] * (BQ // 128), axis=1)
        km = jnp.concatenate([km, km], axis=0)
        sh = (qa_s[fh, DH:2 * DH, :].astype(F32) * km).astype(BF16)
        return jnp.concatenate([qa_s[fh, 0:DH, :], sh, zpad], axis=0)

    def softmax_tile(s):
        p = jnp.exp2(s)
        return p.astype(BF16), p.reshape(BK // 8, 8, BQ).sum(axis=0)

    def handoff(j, s):
        pb, ps = softmax_tile(s)
        p_s[j] = pb
        l_s[j] = ps

    qw0 = q_weights(0)
    for t in range(LA):
        handoff(t, _dot(ka_s[t], qw0))
    for c in c_big:
        c.wait()

    def ssm_in(i, hg, sb):
        xs = jnp.concatenate(
            [x_s[pl.ds(pl.multiple_of(i * BQ + c * TCH + hg * SPI + sb * SUB, SUB), SUB), :]
             for c in range(NCH)], axis=0)
        ur = _dot_nt(xs, bre_s[...])
        ui = _dot_nt(xs, bim_s[...])
        cr = jnp.broadcast_to(coef_s[2, 0:1, :], (NCH * SUB, P))
        ci = jnp.broadcast_to(coef_s[3, 0:1, :], (NCH * SUB, P))
        bur, bui = _cmul(cr, ci, ur, ui)
        for j in range(NP):
            for c in range(NCH):
                dst = slice(c * UPITCH, c * UPITCH + SUB)
                src = slice(c * SUB, (c + 1) * SUB)
                u_s[sb, 0, j, dst, :] = bur[src, j * 128:(j + 1) * 128]
                u_s[sb, 1, j, dst, :] = bui[src, j * 128:(j + 1) * 128]

    def scan_steps(hg, s0, n):
        hr = [st_s[0, j] for j in range(NP)]
        hi = [st_s[1, j] for j in range(NP)]
        for s_ in range(s0, s0 + n):
            t = hg * SPI + s_
            for j in range(NP):
                lr_, li_ = coef_s[0, :, j * 128:(j + 1) * 128], coef_s[1, :, j * 128:(j + 1) * 128]
                a = u_s[s_ // SUB, 0, j, pl.ds(s_ % SUB, NCH, stride=UPITCH), :]
                b = u_s[s_ // SUB, 1, j, pl.ds(s_ % SUB, NCH, stride=UPITCH), :]
                nr_ = lr_ * hr[j] - li_ * hi[j] + a
                ni_ = lr_ * hi[j] + li_ * hr[j] + b
                hr[j], hi[j] = nr_, ni_
                g_s[0, j, pl.ds(t, NCH, stride=PITCH), :] = nr_
                g_s[1, j, pl.ds(t, NCH, stride=PITCH), :] = ni_
        for j in range(NP):
            st_s[0, j] = hr[j]
            st_s[1, j] = hi[j]

    def out_copy(i, r):
        return pltpu.make_async_copy(
            ob_s.at[pl.ds(r * RC, RC)],
            o_hbm.at[pl.ds(pl.multiple_of(i * BQ, BQ) + r * RC, RC)], osem.at[r])

    def qblock(i, _):
        st_s[...] = jnp.zeros_like(st_s)

        def heads_body(hg, bad):
            nst = U * NKB
            slab = nst * SUB // SPI
            qw = {}

            def qk(t):
                u, kb = divmod(t, NKB)
                if u not in qw:
                    fh = i * H + hg * U + u
                    if u == U:
                        fh = jnp.minimum(fh, NB * H - 1)
                    qw[u] = q_weights(fh)
                return _dot(ka_s[kb], qw[u])

            ss = {}
            acc = l8 = None
            for t in range(nst):
                u, kb = divmod(t, NKB)
                if t + LA < nst:
                    ss[t + LA] = qk(t + LA)
                else:
                    handoff(t + LA - nst, qk(t + LA))
                if t < LA:
                    pb, ps = p_s[t], l_s[t]
                else:
                    pb, ps = softmax_tile(ss.pop(t))
                pv = _dot(vt_s[:, kb * BK:(kb + 1) * BK], pb)
                if kb == 0:
                    acc, l8 = pv, ps
                else:
                    acc, l8 = acc + pv, l8 + ps
                if kb == NKB - 1:
                    l = jnp.sum(l8, axis=0, keepdims=True)
                    ot_s[hg * U + u] = acc * (1.0 / l)
                    bad = jnp.maximum(bad, jnp.where(l >= L_MIN, 0.0, 1.0))
                if t % slab == T_SSM:
                    ssm_in(i, hg, t // slab)
                if kb == T_SCAN:
                    scan_steps(hg, u * (SPI // U), SPI // U)
            return bad

        bad = lax.fori_loop(0, NIT, heads_body, jnp.zeros((1, BQ), F32))

        er = jnp.concatenate([st_s[0, j] for j in range(NP)], axis=1)
        ei = jnp.concatenate([st_s[1, j] for j in range(NP)], axis=1)
        c_r, c_i = carry_s[0], carry_s[1]
        tr, ti = _cmul(coef_s[4], coef_s[5], c_r, c_i)
        er = er + jnp.where(row == 0, tr, 0.0)
        ei = ei + jnp.where(row == 0, ti, 0.0)
        for j, d in enumerate((1, 2, 4)):
            sr = jnp.where(row >= d, pltpu.roll(er, d, 0), 0.0)
            si = jnp.where(row >= d, pltpu.roll(ei, d, 0), 0.0)
            tr, ti = _cmul(coef_s[4 + 2 * j], coef_s[5 + 2 * j], sr, si)
            er, ei = er + tr, ei + ti
        carry_s[0] = jnp.broadcast_to(er[NCH - 1:NCH], (NCH, P))
        carry_s[1] = jnp.broadcast_to(ei[NCH - 1:NCH], (NCH, P))
        e0r = jnp.where(row == 0, c_r, pltpu.roll(er, 1, 0))
        e0i = jnp.where(row == 0, c_i, pltpu.roll(ei, 1, 0))

        @pl.when(jnp.max(bad) > 0.0)
        def _exact_softmax():
            def head(h, _):
                qw = jnp.concatenate([qa_s[i * H + h, 0:DH, :], jnp.zeros((128 - DH, BQ), BF16)], axis=0)

                def kb_body(kb, carry):
                    m, l, acc = carry
                    s = _dot(ka_s[kb], qw)
                    m_new = jnp.maximum(m, jnp.max(s, axis=0, keepdims=True))
                    alpha = jnp.exp2(m - m_new)
                    p = jnp.exp2(s - m_new)
                    l = alpha * l + jnp.sum(p, axis=0, keepdims=True)
                    vt = vt_s[:, pl.ds(pl.multiple_of(kb * BK, BK), BK)]
                    acc = alpha * acc + _dot(vt, p.astype(BF16))
                    return m_new, l, acc

                m, l, acc = lax.fori_loop(
                    0, NKB, kb_body,
                    (jnp.full((1, BQ), -jnp.inf, F32), jnp.zeros((1, BQ), F32), jnp.zeros((DH, BQ), F32)))
                ot_s[h] = acc * (1.0 / l)
                return 0

            lax.fori_loop(0, H, head, 0)

        @pl.when(i > 0)
        def _():
            for r in range(BQ // RC):
                out_copy(i - 1, r).wait()

        pwr, pwi = pw_s[0], pw_s[1]
        dsk = coef_s[10, 0:1, :]
        gw = coef_s[11, 0:1, :]
        for r in range(BQ // RC):
            hrs, his = [], []
            for c in range(r * RC // TCH, (r + 1) * RC // TCH):
                rows = slice(c * PITCH, c * PITCH + TCH)
                gr = jnp.concatenate([g_s[0, j, rows, :] for j in range(NP)], axis=1)
                gi = jnp.concatenate([g_s[1, j, rows, :] for j in range(NP)], axis=1)
                br = jnp.broadcast_to(e0r[c:c + 1], (TCH, P))
                bi = jnp.broadcast_to(e0i[c:c + 1], (TCH, P))
                tr, ti = _cmul(pwr, pwi, br, bi)
                hrs.append((gr + tr).astype(BF16))
                his.append((gi + ti).astype(BF16))
            hr = jnp.concatenate(hrs, axis=0)
            hi = jnp.concatenate(his, axis=0)
            y = _dot_nt(hr, cre_s[...]) - _dot_nt(hi, cim_s[...])
            xf = x_s[pl.ds(pl.multiple_of(i * BQ, BQ) + r * RC, RC), :].astype(F32)
            bb = y + xf * dsk
            g = jax.nn.sigmoid(jnp.sum(xf * gw, axis=1, keepdims=True))
            o = ot_s[:, :, r * RC:(r + 1) * RC].reshape(H * DH, RC).T.astype(BF16)
            a = _dot(o, wo_s[...])
            ob_s[r * RC:(r + 1) * RC, :] = g * a + (1.0 - g) * bb
            out_copy(i, r).start()
        return 0

    lax.fori_loop(0, NB, qblock, 0)
    for r in range(BQ // RC):
        out_copy(NB - 1, r).wait()


@jax.jit
def pallas_gated_mix__grouped_kv_mqa__ssm_conv_s5__prompt_kernel(
    A_x, A_wq, A_wk, A_wv, A_wo, B_x, B_Lambda_re, B_Lambda_im, B_B_re, B_B_im,
    B_C_re, B_C_im, B_log_dt, B_Dskip, gate_w,
):
    del B_x
    args = (A_x.reshape(S, D), A_wq, A_wk.T, A_wv.T, A_wo, B_Lambda_re, B_Lambda_im, B_B_re, B_B_im,
            B_C_re, B_C_im, B_log_dt, B_Dskip, gate_w)
    out = pl.pallas_call(
        _kernel,
        in_specs=[pl.BlockSpec(memory_space=pl.ANY)] * len(args),
        out_specs=pl.BlockSpec(memory_space=pl.ANY),
        out_shape=jax.ShapeDtypeStruct((S, D), F32),
        scratch_shapes=[pltpu.VMEM(a.shape, a.dtype) for a in args] + [
            pltpu.VMEM((NB * H, 2 * DH, BQ), BF16),
            pltpu.VMEM((NKB, BK, 128), BF16),
            pltpu.VMEM((DH, S), BF16),
            pltpu.VMEM((8, 128), F32),
            pltpu.VMEM((H, DH, BQ), F32),
            pltpu.VMEM((SPI // SUB, 2, NP, NCH * UPITCH, 128), F32),
            pltpu.VMEM((2, NP, NCH * PITCH, 128), F32),
            pltpu.VMEM((2, NP, NCH, 128), F32),
            pltpu.VMEM((12, 8, P), F32),
            pltpu.VMEM((2, TCH, P), F32),
            pltpu.VMEM((2, 8, P), F32),
            pltpu.VMEM((BQ, D), F32),
            pltpu.VMEM((LA, BK, BQ), BF16),
            pltpu.VMEM((LA, 8, BQ), F32),
            pltpu.SemaphoreType.DMA((13 + NB,)),
            pltpu.SemaphoreType.DMA((BQ // RC,)),
        ],
        compiler_params=pltpu.CompilerParams(vmem_limit_bytes=100 * 1024 * 1024),
        name="gmix",
    )(*args)
    return out.reshape(1, S, D)
```

```python
import numpy as np
import jax
import jax.numpy as jnp
from jax import lax
import jax.experimental.pallas as pl
import jax.experimental.pallas.tpu as pltpu

S, D, H, DH, P = 2048, 512, 32, 16, 512
BQ = 512
NB = S // BQ
SB = 2
NSB = NB // SB
BK = 128
NKB = S // BK
LA = 2
U = 16
NIT = SB * H // U
NCH = 8
TCH = SB * BQ // NCH
SPI = TCH // NIT
SUB = 16
PITCH = TCH + 8
UPITCH = SUB + 8
NP = P // 128
RC = 128
T_SSM = 2
T_SCAN = NKB // 2
QSCALE = float(np.log2(np.e) * DH ** -0.5)
UP = 1.0 + 2.0 ** -7
L_MIN = 2.0 ** -64
F32, BF16 = jnp.float32, jnp.bfloat16
NT = (((1,), (1,)), ((), ()))


def _dot(a, b):
    return jnp.dot(a, b, preferred_element_type=F32)


def _dot_nt(a, b):
    return lax.dot_general(a, b, NT, preferred_element_type=F32)


def _cmul(ar, ai, br, bi):
    return ar * br - ai * bi, ar * bi + ai * br


def _kernel(x_hbm, wq_hbm, wk_hbm, wv_hbm, wo_hbm, lre_hbm, lim_hbm, bre_hbm, bim_hbm,
            cre_hbm, cim_hbm, ldt_hbm, dsk_hbm, gw_hbm, o_hbm,
            x_s, wq_s, wk_s, wv_s, wo_s, lre_s, lim_s, bre_s, bim_s, cre_s, cim_s, ldt_s, dsk_s, gw_s,
            qa_s, ka_s, vt_s, km_s, ot_s, u_s, g_s, st_s, coef_s, pw_s, carry_s, ob_s, p_s, l_s,
            isem, osem):
    def cp(src, dst, n):
        return pltpu.make_async_copy(src, dst, isem.at[n])

    c_wq, c_wk, c_wv = cp(wq_hbm, wq_s, 0), cp(wk_hbm, wk_s, 1), cp(wv_hbm, wv_s, 2)
    c_x = [cp(x_hbm.at[pl.ds(t * BQ, BQ)], x_s.at[pl.ds(t * BQ, BQ)], 3 + t) for t in range(NB)]
    c_vec = [cp(a, b, 3 + NB + n) for n, (a, b) in enumerate(
        ((lre_hbm, lre_s), (lim_hbm, lim_s), (ldt_hbm, ldt_s), (dsk_hbm, dsk_s), (gw_hbm, gw_s)))]
    c_big = [cp(a, b, 8 + NB + n) for n, (a, b) in enumerate(
        ((bre_hbm, bre_s), (bim_hbm, bim_s), (cre_hbm, cre_s), (cim_hbm, cim_s), (wo_hbm, wo_s)))]
    for c in c_vec + [c_wq, c_wk, c_wv] + c_x + c_big:
        c.start()

    for c in c_vec:
        c.wait()

    def vec8(ref):
        return jnp.broadcast_to(ref[...].astype(F32).reshape(1, P), (8, P))

    lre, lim = vec8(lre_s), vec8(lim_s)
    dt = jnp.exp(vec8(ldt_s)).astype(BF16).astype(F32)
    er = jnp.exp(dt * lre)
    lr = er * jnp.cos(dt * lim)
    li = er * jnp.sin(dt * lim)
    den = lre * lre + lim * lim
    nr = lr - 1.0
    coef_s[0] = lr
    coef_s[1] = li
    coef_s[2] = 2.0 * (nr * lre + li * lim) / den
    coef_s[3] = 2.0 * (li * lre - nr * lim) / den
    row = lax.broadcasted_iota(jnp.int32, (NCH, P), 0)
    pr, pi = lr, li
    ar, ai = lr, li
    for k in range(3):
        tr, ti = _cmul(pr, pi, ar, ai)
        sel = (row & (1 << k)) != 0
        pr, pi = jnp.where(sel, tr, pr), jnp.where(sel, ti, pi)
        ar, ai = _cmul(ar, ai, ar, ai)
    for g in range(TCH // 8):
        pw_s[0, g * 8:(g + 1) * 8, :] = pr
        pw_s[1, g * 8:(g + 1) * 8, :] = pi
        pr, pi = _cmul(pr, pi, ar, ai)
    for _ in range(TCH.bit_length() - 4):
        ar, ai = _cmul(ar, ai, ar, ai)
    for j in range(3):
        coef_s[4 + 2 * j] = ar
        coef_s[5 + 2 * j] = ai
        ar, ai = _cmul(ar, ai, ar, ai)
    coef_s[10] = vec8(dsk_s)
    coef_s[11] = vec8(gw_s)
    carry_s[...] = jnp.zeros_like(carry_s)

    c_wq.wait()
    c_wk.wait()
    c_wv.wait()
    c_x[0].wait()
    wqT = wq_s[...].astype(F32).T.astype(BF16)
    lhs = jnp.concatenate([wk_s[...], wv_s[...], wqT], axis=0)
    k2max = None
    for tb in range(NB):
        if tb == 1:
            c_x[1].wait()
        if tb == 2:
            for c in c_x[2:]:
                c.wait()
        r = _dot_nt(lhs, x_s[tb * BQ:(tb + 1) * BQ, :])
        q = (r[2 * DH:] * QSCALE).astype(BF16)
        qf = q.astype(F32)
        for h in range(H):
            a = qf[h * DH:h * DH + 8]
            b = qf[h * DH + 8:(h + 1) * DH]
            n = a * a + b * b
            n = n + pltpu.roll(n, 4, 0)
            n = n + pltpu.roll(n, 2, 0)
            n = n + pltpu.roll(n, 1, 0)
            nrm = -(jnp.sqrt(n) * UP)
            qa_s[tb * H + h, 0:DH, :] = q[h * DH:(h + 1) * DH]
            qa_s[tb * H + h, DH:2 * DH, :] = jnp.concatenate([nrm, nrm], axis=0).astype(BF16)
        kt = r[0:DH].astype(BF16).astype(F32)
        vt_s[:, tb * BQ:(tb + 1) * BQ] = r[DH:2 * DH].astype(BF16)
        k2 = jnp.sum(kt * kt, axis=0, keepdims=True)
        k2max = k2 if k2max is None else jnp.maximum(k2max, k2)
        for kb in range(BQ // BK):
            kta = jnp.concatenate([kt[:, kb * BK:(kb + 1) * BK],
                                   jnp.full((DH, BK), 1.0 / DH, F32),
                                   jnp.zeros((128 - 2 * DH, BK), F32)], axis=0)
            ka_s[tb * (BQ // BK) + kb] = kta.T.astype(BF16)
    kmax = jnp.sqrt(jnp.max(k2max, axis=1, keepdims=True)) * UP
    km_s[...] = jnp.broadcast_to(kmax, (8, 128))

    zpad = jnp.zeros((128 - 2 * DH, BQ), BF16)

    def q_weights(fh):
        km = jnp.concatenate([km_s[...]] * (BQ // 128), axis=1)
        km = jnp.concatenate([km, km], axis=0)
        sh = (qa_s[fh, DH:2 * DH, :].astype(F32) * km).astype(BF16)
        return jnp.concatenate([qa_s[fh, 0:DH, :], sh, zpad], axis=0)

    def softmax_tile(s):
        p = jnp.exp2(s)
        return p.astype(BF16), p.reshape(BK // 8, 8, BQ).sum(axis=0)

    def handoff(j, s):
        pb, ps = softmax_tile(s)
        p_s[j] = pb
        l_s[j] = ps

    qw0 = q_weights(0)
    for t in range(LA):
        handoff(t, _dot(ka_s[t], qw0))
    for c in c_big:
        c.wait()

    def ssm_in(i, hg, sb):
        xs = jnp.concatenate(
            [x_s[pl.ds(pl.multiple_of(i * (SB * BQ) + c * TCH + hg * SPI + sb * SUB, SUB), SUB), :]
             for c in range(NCH)], axis=0)
        ur = _dot_nt(xs, bre_s[...])
        ui = _dot_nt(xs, bim_s[...])
        cr = jnp.broadcast_to(coef_s[2, 0:1, :], (NCH * SUB, P))
        ci = jnp.broadcast_to(coef_s[3, 0:1, :], (NCH * SUB, P))
        bur, bui = _cmul(cr, ci, ur, ui)
        for j in range(NP):
            for c in range(NCH):
                dst = slice(c * UPITCH, c * UPITCH + SUB)
                src = slice(c * SUB, (c + 1) * SUB)
                u_s[sb, 0, j, dst, :] = bur[src, j * 128:(j + 1) * 128]
                u_s[sb, 1, j, dst, :] = bui[src, j * 128:(j + 1) * 128]

    def scan_steps(hg, s0, n):
        hr = [st_s[0, j] for j in range(NP)]
        hi = [st_s[1, j] for j in range(NP)]
        for s_ in range(s0, s0 + n):
            t = hg * SPI + s_
            for j in range(NP):
                lr_, li_ = coef_s[0, :, j * 128:(j + 1) * 128], coef_s[1, :, j * 128:(j + 1) * 128]
                a = u_s[s_ // SUB, 0, j, pl.ds(s_ % SUB, NCH, stride=UPITCH), :]
                b = u_s[s_ // SUB, 1, j, pl.ds(s_ % SUB, NCH, stride=UPITCH), :]
                nr_ = lr_ * hr[j] - li_ * hi[j] + a
                ni_ = lr_ * hi[j] + li_ * hr[j] + b
                hr[j], hi[j] = nr_, ni_
                g_s[0, j, pl.ds(t, NCH, stride=PITCH), :] = nr_
                g_s[1, j, pl.ds(t, NCH, stride=PITCH), :] = ni_
        for j in range(NP):
            st_s[0, j] = hr[j]
            st_s[1, j] = hi[j]

    def out_copy(i, r):
        return pltpu.make_async_copy(
            ob_s.at[pl.ds(r * RC, RC)],
            o_hbm.at[pl.ds(pl.multiple_of(i * (SB * BQ), BQ) + r * RC, RC)], osem.at[r])

    def qblock(i, _):
        st_s[...] = jnp.zeros_like(st_s)

        def heads_body(hg, bad):
            nst = U * NKB
            slab = nst * SUB // SPI
            qw = {}

            def qk(t):
                u, kb = divmod(t, NKB)
                if u not in qw:
                    fh = i * (SB * H) + hg * U + u
                    if u == U:
                        fh = jnp.minimum(fh, NB * H - 1)
                    qw[u] = q_weights(fh)
                return _dot(ka_s[kb], qw[u])

            ss = {}
            acc = l8 = None
            for t in range(nst):
                u, kb = divmod(t, NKB)
                if t + LA < nst:
                    ss[t + LA] = qk(t + LA)
                else:
                    handoff(t + LA - nst, qk(t + LA))
                if t < LA:
                    pb, ps = p_s[t], l_s[t]
                else:
                    pb, ps = softmax_tile(ss.pop(t))
                pv = _dot(vt_s[:, kb * BK:(kb + 1) * BK], pb)
                if kb == 0:
                    acc, l8 = pv, ps
                else:
                    acc, l8 = acc + pv, l8 + ps
                if kb == NKB - 1:
                    l = jnp.sum(l8, axis=0, keepdims=True)
                    ot_s[hg * U + u] = acc * (1.0 / l)
                    bad = jnp.maximum(bad, jnp.where(l >= L_MIN, 0.0, 1.0))
                if t % slab == T_SSM:
                    ssm_in(i, hg, t // slab)
                if kb == T_SCAN:
                    scan_steps(hg, u * (SPI // U), SPI // U)
            return bad

        bad = lax.fori_loop(0, NIT, heads_body, jnp.zeros((1, BQ), F32))

        er = jnp.concatenate([st_s[0, j] for j in range(NP)], axis=1)
        ei = jnp.concatenate([st_s[1, j] for j in range(NP)], axis=1)
        c_r, c_i = carry_s[0], carry_s[1]
        tr, ti = _cmul(coef_s[4], coef_s[5], c_r, c_i)
        er = er + jnp.where(row == 0, tr, 0.0)
        ei = ei + jnp.where(row == 0, ti, 0.0)
        for j, d in enumerate((1, 2, 4)):
            sr = jnp.where(row >= d, pltpu.roll(er, d, 0), 0.0)
            si = jnp.where(row >= d, pltpu.roll(ei, d, 0), 0.0)
            tr, ti = _cmul(coef_s[4 + 2 * j], coef_s[5 + 2 * j], sr, si)
            er, ei = er + tr, ei + ti
        carry_s[0] = jnp.broadcast_to(er[NCH - 1:NCH], (NCH, P))
        carry_s[1] = jnp.broadcast_to(ei[NCH - 1:NCH], (NCH, P))
        e0r = jnp.where(row == 0, c_r, pltpu.roll(er, 1, 0))
        e0i = jnp.where(row == 0, c_i, pltpu.roll(ei, 1, 0))

        @pl.when(jnp.max(bad) > 0.0)
        def _exact_softmax():
            def head(h, _):
                qw = jnp.concatenate([qa_s[i * (SB * H) + h, 0:DH, :], jnp.zeros((128 - DH, BQ), BF16)], axis=0)

                def kb_body(kb, carry):
                    m, l, acc = carry
                    s = _dot(ka_s[kb], qw)
                    m_new = jnp.maximum(m, jnp.max(s, axis=0, keepdims=True))
                    alpha = jnp.exp2(m - m_new)
                    p = jnp.exp2(s - m_new)
                    l = alpha * l + jnp.sum(p, axis=0, keepdims=True)
                    vt = vt_s[:, pl.ds(pl.multiple_of(kb * BK, BK), BK)]
                    acc = alpha * acc + _dot(vt, p.astype(BF16))
                    return m_new, l, acc

                m, l, acc = lax.fori_loop(
                    0, NKB, kb_body,
                    (jnp.full((1, BQ), -jnp.inf, F32), jnp.zeros((1, BQ), F32), jnp.zeros((DH, BQ), F32)))
                ot_s[h] = acc * (1.0 / l)
                return 0

            lax.fori_loop(0, SB * H, head, 0)

        @pl.when(i > 0)
        def _():
            for r in range(SB * BQ // RC):
                out_copy(i - 1, r).wait()

        pwr, pwi = pw_s[0], pw_s[1]
        dsk = coef_s[10, 0:1, :]
        gw = coef_s[11, 0:1, :]
        for r in range(SB * BQ // RC):
            hrs, his = [], []
            for c in range(r * RC // TCH, (r + 1) * RC // TCH):
                rows = slice(c * PITCH, c * PITCH + TCH)
                gr = jnp.concatenate([g_s[0, j, rows, :] for j in range(NP)], axis=1)
                gi = jnp.concatenate([g_s[1, j, rows, :] for j in range(NP)], axis=1)
                br = jnp.broadcast_to(e0r[c:c + 1], (TCH, P))
                bi = jnp.broadcast_to(e0i[c:c + 1], (TCH, P))
                tr, ti = _cmul(pwr, pwi, br, bi)
                hrs.append((gr + tr).astype(BF16))
                his.append((gi + ti).astype(BF16))
            hr = jnp.concatenate(hrs, axis=0)
            hi = jnp.concatenate(his, axis=0)
            y = _dot_nt(hr, cre_s[...]) - _dot_nt(hi, cim_s[...])
            xf = x_s[pl.ds(pl.multiple_of(i * (SB * BQ), BQ) + r * RC, RC), :].astype(F32)
            bb = y + xf * dsk
            g = jax.nn.sigmoid(jnp.sum(xf * gw, axis=1, keepdims=True))
            hb, lo = divmod(r * RC, BQ)
            o = ot_s[hb * H:(hb + 1) * H, :, lo:lo + RC].reshape(H * DH, RC).T.astype(BF16)
            a = _dot(o, wo_s[...])
            ob_s[r * RC:(r + 1) * RC, :] = g * a + (1.0 - g) * bb
            out_copy(i, r).start()
        return 0

    lax.fori_loop(0, NSB, qblock, 0)
    for r in range(SB * BQ // RC):
        out_copy(NSB - 1, r).wait()


@jax.jit
def pallas_gated_mix__grouped_kv_mqa__ssm_conv_s5__prompt_kernel(
    A_x, A_wq, A_wk, A_wv, A_wo, B_x, B_Lambda_re, B_Lambda_im, B_B_re, B_B_im,
    B_C_re, B_C_im, B_log_dt, B_Dskip, gate_w,
):
    del B_x
    args = (A_x.reshape(S, D), A_wq, A_wk.T, A_wv.T, A_wo, B_Lambda_re, B_Lambda_im, B_B_re, B_B_im,
            B_C_re, B_C_im, B_log_dt, B_Dskip, gate_w)
    out = pl.pallas_call(
        _kernel,
        in_specs=[pl.BlockSpec(memory_space=pl.ANY)] * len(args),
        out_specs=pl.BlockSpec(memory_space=pl.ANY),
        out_shape=jax.ShapeDtypeStruct((S, D), F32),
        scratch_shapes=[pltpu.VMEM(a.shape, a.dtype) for a in args] + [
            pltpu.VMEM((NB * H, 2 * DH, BQ), BF16),
            pltpu.VMEM((NKB, BK, 128), BF16),
            pltpu.VMEM((DH, S), BF16),
            pltpu.VMEM((8, 128), F32),
            pltpu.VMEM((SB * H, DH, BQ), F32),
            pltpu.VMEM((SPI // SUB, 2, NP, NCH * UPITCH, 128), F32),
            pltpu.VMEM((2, NP, NCH * PITCH, 128), F32),
            pltpu.VMEM((2, NP, NCH, 128), F32),
            pltpu.VMEM((12, 8, P), F32),
            pltpu.VMEM((2, TCH, P), F32),
            pltpu.VMEM((2, 8, P), F32),
            pltpu.VMEM((SB * BQ, D), F32),
            pltpu.VMEM((LA, BK, BQ), BF16),
            pltpu.VMEM((LA, 8, BQ), F32),
            pltpu.SemaphoreType.DMA((13 + NB,)),
            pltpu.SemaphoreType.DMA((SB * BQ // RC,)),
        ],
        compiler_params=pltpu.CompilerParams(vmem_limit_bytes=100 * 1024 * 1024),
        name="gmix",
    )(*args)
    return out.reshape(1, S, D)
```

```python
import numpy as np
import jax
import jax.numpy as jnp
from jax import lax
import jax.experimental.pallas as pl
import jax.experimental.pallas.tpu as pltpu

S, D, H, DH, P = 2048, 512, 32, 16, 512
BQ = 512
NB = S // BQ
SB = 2
NSB = NB // SB
BK = 128
NKB = S // BK
LA = 2
U = 16
NIT = SB * H // U
NCH = 8
TCH = SB * BQ // NCH
SPI = TCH // NIT
SUB = 16
PITCH = TCH + 8
UPITCH = SUB + 8
NP = P // 128
NH = 2
RC = 128
N_ISEM = 12 + 2 * NH + NB - 1
T_SSM = 2
T_SCAN = NKB // 2
QSCALE = float(np.log2(np.e) * DH ** -0.5)
UP = 1.0 + 2.0 ** -7
L_MIN = 2.0 ** -64
L_MAX = 2.0 ** 64
F32, BF16 = jnp.float32, jnp.bfloat16
NT = (((1,), (1,)), ((), ()))


def _dot(a, b):
    return jnp.dot(a, b, preferred_element_type=F32)


def _dot_nt(a, b):
    return lax.dot_general(a, b, NT, preferred_element_type=F32)


def _cmul(ar, ai, br, bi):
    return ar * br - ai * bi, ar * bi + ai * br


def _kernel(x_hbm, wq_hbm, wk_hbm, wv_hbm, wo_hbm, lre_hbm, lim_hbm, bre_hbm, bim_hbm,
            cre_hbm, cim_hbm, ldt_hbm, dsk_hbm, gw_hbm, o_hbm,
            x_s, wq_s, wk_s, wv_s, wo_s, lre_s, lim_s, bre_s, bim_s, cre_s, cim_s, ldt_s, dsk_s, gw_s,
            qa_s, ka_s, vt_s, km_s, ot_s, u_s, g_s, st_s, coef_s, pw_s, carry_s, ob_s, p_s, l_s, r_s,
            isem, osem):
    def cp(src, dst):
        return pltpu.make_async_copy(src, dst, isem.at[next(sems)])

    HD = D // NH
    sems = iter(range(N_ISEM))
    c_wk, c_wv = cp(wk_hbm, wk_s), cp(wv_hbm, wv_s)
    c_piece = [[cp(wq_hbm.at[pl.ds(h * HD, HD)], wq_s.at[pl.ds(h * HD, HD)]),
                cp(x_hbm.at[pl.ds(0, BQ), pl.ds(h * HD, HD)], x_s.at[pl.ds(0, BQ), pl.ds(h * HD, HD)])]
               for h in range(NH)]
    c_x = [cp(x_hbm.at[pl.ds(t * BQ, BQ)], x_s.at[pl.ds(t * BQ, BQ)]) for t in range(1, NB)]
    c_vec = [cp(a, b) for a, b in
             ((lre_hbm, lre_s), (lim_hbm, lim_s), (ldt_hbm, ldt_s), (dsk_hbm, dsk_s), (gw_hbm, gw_s))]
    c_big = [cp(a, b) for a, b in
             ((bre_hbm, bre_s), (bim_hbm, bim_s), (cre_hbm, cre_s), (cim_hbm, cim_s), (wo_hbm, wo_s))]
    for c in c_vec + [c_wk, c_wv] + sum(c_piece, []) + c_x + c_big:
        c.start()

    for c in c_vec:
        c.wait()

    def vec8(ref):
        return jnp.broadcast_to(ref[...].astype(F32).reshape(1, P), (8, P))

    lre, lim = vec8(lre_s), vec8(lim_s)
    dt = jnp.exp(vec8(ldt_s)).astype(BF16).astype(F32)
    er = jnp.exp(dt * lre)
    lr = er * jnp.cos(dt * lim)
    li = er * jnp.sin(dt * lim)
    den = lre * lre + lim * lim
    nr = lr - 1.0
    coef_s[0] = lr
    coef_s[1] = li
    coef_s[2] = 2.0 * (nr * lre + li * lim) / den
    coef_s[3] = 2.0 * (li * lre - nr * lim) / den
    row = lax.broadcasted_iota(jnp.int32, (NCH, P), 0)
    pr, pi = lr, li
    ar, ai = lr, li
    for k in range(3):
        tr, ti = _cmul(pr, pi, ar, ai)
        sel = (row & (1 << k)) != 0
        pr, pi = jnp.where(sel, tr, pr), jnp.where(sel, ti, pi)
        ar, ai = _cmul(ar, ai, ar, ai)
    for g in range(TCH // 8):
        pw_s[0, g * 8:(g + 1) * 8, :] = pr
        pw_s[1, g * 8:(g + 1) * 8, :] = pi
        pr, pi = _cmul(pr, pi, ar, ai)
    for _ in range(TCH.bit_length() - 4):
        ar, ai = _cmul(ar, ai, ar, ai)
    for j in range(3):
        coef_s[4 + 2 * j] = ar
        coef_s[5 + 2 * j] = ai
        ar, ai = _cmul(ar, ai, ar, ai)
    coef_s[10] = vec8(dsk_s)
    coef_s[11] = vec8(gw_s)
    carry_s[...] = jnp.zeros_like(carry_s)

    c_wk.wait()
    c_wv.wait()
    lhs_h = []
    for h in range(NH):
        for c in c_piece[h]:
            c.wait()
        ks = slice(h * HD, (h + 1) * HD)
        wqT = wq_s[ks, :].astype(F32).T.astype(BF16)
        lhs_h.append(jnp.concatenate([wk_s[:, ks], wv_s[:, ks], wqT], axis=0))
        part = _dot_nt(lhs_h[h], x_s[0:BQ, ks])
        if h == 0:
            r_s[...] = part
        elif h < NH - 1:
            r_s[...] = r_s[...] + part
        else:
            r0 = r_s[...] + part
    lhs = jnp.concatenate(lhs_h, axis=1)
    k2max = None
    for tb in range(NB):
        if tb == 1:
            c_x[0].wait()
        if tb == 2:
            for c in c_x[1:]:
                c.wait()
        r = r0 if tb == 0 else _dot_nt(lhs, x_s[tb * BQ:(tb + 1) * BQ, :])
        q = (r[2 * DH:] * QSCALE).astype(BF16)
        qf = q.astype(F32)
        for h in range(H):
            a = qf[h * DH:h * DH + 8]
            b = qf[h * DH + 8:(h + 1) * DH]
            n = a * a + b * b
            n = n + pltpu.roll(n, 4, 0)
            n = n + pltpu.roll(n, 2, 0)
            n = n + pltpu.roll(n, 1, 0)
            nrm = -(jnp.sqrt(n) * UP)
            qa_s[tb * H + h, 0:DH, :] = q[h * DH:(h + 1) * DH]
            qa_s[tb * H + h, DH:2 * DH, :] = jnp.concatenate([nrm, nrm], axis=0).astype(BF16)
        kt = r[0:DH].astype(BF16).astype(F32)
        vt_s[:, tb * BQ:(tb + 1) * BQ] = r[DH:2 * DH].astype(BF16)
        k2 = jnp.sum(kt * kt, axis=0, keepdims=True)
        k2max = k2 if k2max is None else jnp.maximum(k2max, k2)
        for kb in range(BQ // BK):
            kta = jnp.concatenate([kt[:, kb * BK:(kb + 1) * BK],
                                   jnp.full((DH, BK), 1.0 / DH, F32),
                                   jnp.zeros((128 - 2 * DH, BK), F32)], axis=0)
            ka_s[tb * (BQ // BK) + kb] = kta.T.astype(BF16)
    kmax = jnp.sqrt(jnp.max(k2max, axis=1, keepdims=True)) * UP
    km_s[...] = jnp.broadcast_to(kmax, (8, 128))

    zpad = jnp.zeros((128 - 2 * DH, BQ), BF16)

    def q_weights(fh):
        km = jnp.concatenate([km_s[...]] * (BQ // 128), axis=1)
        km = jnp.concatenate([km, km], axis=0)
        sh = (qa_s[fh, DH:2 * DH, :].astype(F32) * km).astype(BF16)
        return jnp.concatenate([qa_s[fh, 0:DH, :], sh, zpad], axis=0)

    def softmax_tile(s):
        p = jnp.exp2(s)
        return p.astype(BF16), p.reshape(BK // 8, 8, BQ).sum(axis=0)

    def handoff(j, s):
        pb, ps = softmax_tile(s)
        p_s[j] = pb
        l_s[j] = ps

    qw0 = q_weights(0)
    for t in range(LA):
        handoff(t, _dot(ka_s[t], qw0))
    for c in c_big:
        c.wait()

    def ssm_in(i, hg, sb):
        xs = jnp.concatenate(
            [x_s[pl.ds(pl.multiple_of(i * (SB * BQ) + c * TCH + hg * SPI + sb * SUB, SUB), SUB), :]
             for c in range(NCH)], axis=0)
        ur = _dot_nt(xs, bre_s[...])
        ui = _dot_nt(xs, bim_s[...])
        cr = jnp.broadcast_to(coef_s[2, 0:1, :], (NCH * SUB, P))
        ci = jnp.broadcast_to(coef_s[3, 0:1, :], (NCH * SUB, P))
        bur, bui = _cmul(cr, ci, ur, ui)
        for j in range(NP):
            for c in range(NCH):
                dst = slice(c * UPITCH, c * UPITCH + SUB)
                src = slice(c * SUB, (c + 1) * SUB)
                u_s[sb, 0, j, dst, :] = bur[src, j * 128:(j + 1) * 128]
                u_s[sb, 1, j, dst, :] = bui[src, j * 128:(j + 1) * 128]

    def scan_steps(hg, s0, n):
        hr = [st_s[0, j] for j in range(NP)]
        hi = [st_s[1, j] for j in range(NP)]
        for s_ in range(s0, s0 + n):
            t = hg * SPI + s_
            for j in range(NP):
                lr_, li_ = coef_s[0, :, j * 128:(j + 1) * 128], coef_s[1, :, j * 128:(j + 1) * 128]
                a = u_s[s_ // SUB, 0, j, pl.ds(s_ % SUB, NCH, stride=UPITCH), :]
                b = u_s[s_ // SUB, 1, j, pl.ds(s_ % SUB, NCH, stride=UPITCH), :]
                nr_ = lr_ * hr[j] - li_ * hi[j] + a
                ni_ = lr_ * hi[j] + li_ * hr[j] + b
                hr[j], hi[j] = nr_, ni_
                g_s[0, j, pl.ds(t, NCH, stride=PITCH), :] = nr_
                g_s[1, j, pl.ds(t, NCH, stride=PITCH), :] = ni_
        for j in range(NP):
            st_s[0, j] = hr[j]
            st_s[1, j] = hi[j]

    def out_copy(i, r):
        return pltpu.make_async_copy(
            ob_s.at[pl.ds(r * RC, RC)],
            o_hbm.at[pl.ds(pl.multiple_of(i * (SB * BQ), BQ) + r * RC, RC)], osem.at[r])

    def qblock(i, _):
        st_s[...] = jnp.zeros_like(st_s)

        def heads_body(hg, bad):
            nst = U * NKB
            slab = nst * SUB // SPI
            qw = {}

            def qk(t):
                u, kb = divmod(t, NKB)
                if u not in qw:
                    fh = i * (SB * H) + hg * U + u
                    if u == U:
                        fh = jnp.minimum(fh, NB * H - 1)
                    qw[u] = q_weights(fh)
                return _dot(ka_s[kb], qw[u])

            ss = {}
            acc = l8 = None
            for t in range(nst):
                u, kb = divmod(t, NKB)
                if t + LA < nst:
                    ss[t + LA] = qk(t + LA)
                else:
                    handoff(t + LA - nst, qk(t + LA))
                if t < LA:
                    pb, ps = p_s[t], l_s[t]
                else:
                    pb, ps = softmax_tile(ss.pop(t))
                pv = _dot(vt_s[:, kb * BK:(kb + 1) * BK], pb)
                if kb == 0:
                    acc, l8 = pv, ps
                else:
                    acc, l8 = acc + pv, l8 + ps
                if kb == NKB - 1:
                    l = jnp.sum(l8, axis=0, keepdims=True)
                    ot_s[hg * U + u] = acc * (1.0 / l)
                    bad = jnp.maximum(bad, jnp.where((l >= L_MIN) & (l <= L_MAX), 0.0, 1.0))
                if t % slab == T_SSM:
                    ssm_in(i, hg, t // slab)
                if kb == T_SCAN:
                    scan_steps(hg, u * (SPI // U), SPI // U)
            return bad

        bad = lax.fori_loop(0, NIT, heads_body, jnp.zeros((1, BQ), F32))

        er = jnp.concatenate([st_s[0, j] for j in range(NP)], axis=1)
        ei = jnp.concatenate([st_s[1, j] for j in range(NP)], axis=1)
        c_r, c_i = carry_s[0], carry_s[1]
        tr, ti = _cmul(coef_s[4], coef_s[5], c_r, c_i)
        er = er + jnp.where(row == 0, tr, 0.0)
        ei = ei + jnp.where(row == 0, ti, 0.0)
        for j, d in enumerate((1, 2, 4)):
            sr = jnp.where(row >= d, pltpu.roll(er, d, 0), 0.0)
            si = jnp.where(row >= d, pltpu.roll(ei, d, 0), 0.0)
            tr, ti = _cmul(coef_s[4 + 2 * j], coef_s[5 + 2 * j], sr, si)
            er, ei = er + tr, ei + ti
        carry_s[0] = jnp.broadcast_to(er[NCH - 1:NCH], (NCH, P))
        carry_s[1] = jnp.broadcast_to(ei[NCH - 1:NCH], (NCH, P))
        e0r = jnp.where(row == 0, c_r, pltpu.roll(er, 1, 0))
        e0i = jnp.where(row == 0, c_i, pltpu.roll(ei, 1, 0))

        @pl.when(jnp.max(bad) > 0.0)
        def _exact_softmax():
            def head(h, _):
                qw = jnp.concatenate([qa_s[i * (SB * H) + h, 0:DH, :], jnp.zeros((128 - DH, BQ), BF16)], axis=0)

                def kb_body(kb, carry):
                    m, l, acc = carry
                    s = _dot(ka_s[kb], qw)
                    m_new = jnp.maximum(m, jnp.max(s, axis=0, keepdims=True))
                    alpha = jnp.exp2(m - m_new)
                    p = jnp.exp2(s - m_new)
                    l = alpha * l + jnp.sum(p, axis=0, keepdims=True)
                    vt = vt_s[:, pl.ds(pl.multiple_of(kb * BK, BK), BK)]
                    acc = alpha * acc + _dot(vt, p.astype(BF16))
                    return m_new, l, acc

                m, l, acc = lax.fori_loop(
                    0, NKB, kb_body,
                    (jnp.full((1, BQ), -jnp.inf, F32), jnp.zeros((1, BQ), F32), jnp.zeros((DH, BQ), F32)))
                ot_s[h] = acc * (1.0 / l)
                return 0

            lax.fori_loop(0, SB * H, head, 0)

        @pl.when(i > 0)
        def _():
            for r in range(SB * BQ // RC):
                out_copy(i - 1, r).wait()

        pwr, pwi = pw_s[0], pw_s[1]
        dsk = coef_s[10, 0:1, :]
        gw = coef_s[11, 0:1, :]
        for r in range(SB * BQ // RC):
            hrs, his = [], []
            for c in range(r * RC // TCH, (r + 1) * RC // TCH):
                rows = slice(c * PITCH, c * PITCH + TCH)
                gr = jnp.concatenate([g_s[0, j, rows, :] for j in range(NP)], axis=1)
                gi = jnp.concatenate([g_s[1, j, rows, :] for j in range(NP)], axis=1)
                br = jnp.broadcast_to(e0r[c:c + 1], (TCH, P))
                bi = jnp.broadcast_to(e0i[c:c + 1], (TCH, P))
                tr, ti = _cmul(pwr, pwi, br, bi)
                hrs.append((gr + tr).astype(BF16))
                his.append((gi + ti).astype(BF16))
            hr = jnp.concatenate(hrs, axis=0)
            hi = jnp.concatenate(his, axis=0)
            y = _dot_nt(hr, cre_s[...]) - _dot_nt(hi, cim_s[...])
            xf = x_s[pl.ds(pl.multiple_of(i * (SB * BQ), BQ) + r * RC, RC), :].astype(F32)
            bb = y + xf * dsk
            g = jax.nn.sigmoid(jnp.sum(xf * gw, axis=1, keepdims=True))
            hb, lo = divmod(r * RC, BQ)
            o = ot_s[hb * H:(hb + 1) * H, :, lo:lo + RC].reshape(H * DH, RC).T.astype(BF16)
            a = _dot(o, wo_s[...])
            ob_s[r * RC:(r + 1) * RC, :] = g * a + (1.0 - g) * bb
            out_copy(i, r).start()
        return 0

    lax.fori_loop(0, NSB, qblock, 0)
    for r in range(SB * BQ // RC):
        out_copy(NSB - 1, r).wait()


@jax.jit
def pallas_gated_mix__grouped_kv_mqa__ssm_conv_s5__prompt_kernel(
    A_x, A_wq, A_wk, A_wv, A_wo, B_x, B_Lambda_re, B_Lambda_im, B_B_re, B_B_im,
    B_C_re, B_C_im, B_log_dt, B_Dskip, gate_w,
):
    del B_x
    args = (A_x.reshape(S, D), A_wq, A_wk.T, A_wv.T, A_wo, B_Lambda_re, B_Lambda_im, B_B_re, B_B_im,
            B_C_re, B_C_im, B_log_dt, B_Dskip, gate_w)
    out = pl.pallas_call(
        _kernel,
        in_specs=[pl.BlockSpec(memory_space=pl.ANY)] * len(args),
        out_specs=pl.BlockSpec(memory_space=pl.ANY),
        out_shape=jax.ShapeDtypeStruct((S, D), F32),
        scratch_shapes=[pltpu.VMEM(a.shape, a.dtype) for a in args] + [
            pltpu.VMEM((NB * H, 2 * DH, BQ), BF16),
            pltpu.VMEM((NKB, BK, 128), BF16),
            pltpu.VMEM((DH, S), BF16),
            pltpu.VMEM((8, 128), F32),
            pltpu.VMEM((SB * H, DH, BQ), F32),
            pltpu.VMEM((SPI // SUB, 2, NP, NCH * UPITCH, 128), F32),
            pltpu.VMEM((2, NP, NCH * PITCH, 128), F32),
            pltpu.VMEM((2, NP, NCH, 128), F32),
            pltpu.VMEM((12, 8, P), F32),
            pltpu.VMEM((2, TCH, P), F32),
            pltpu.VMEM((2, 8, P), F32),
            pltpu.VMEM((SB * BQ, D), F32),
            pltpu.VMEM((LA, BK, BQ), BF16),
            pltpu.VMEM((LA, 8, BQ), F32),
            pltpu.VMEM((D + 2 * DH, BQ), F32),
            pltpu.SemaphoreType.DMA((N_ISEM,)),
            pltpu.SemaphoreType.DMA((SB * BQ // RC,)),
        ],
        compiler_params=pltpu.CompilerParams(vmem_limit_bytes=100 * 1024 * 1024),
        name="gmix",
    )(*args)
    return out.reshape(1, S, D)
```
